```python
import os as _os
_os.environ.setdefault("JAX_PLATFORMS", "cpu")
import jax
import jax.numpy as jnp

def _softmax(x, axis=-1):
    return jax.nn.softmax(x, axis=axis)
def _gelu(x):
    return jax.nn.gelu(x, approximate=True)
def _silu(x):
    return jax.nn.silu(x)
def _sigmoid(x):
    return jax.nn.sigmoid(x)
def _layernorm(x, axis=-1, eps=1e-5):
    m = jnp.mean(x, axis=axis, keepdims=True)
    v = jnp.var(x, axis=axis, keepdims=True)
    return (x - m) / jnp.sqrt(v + eps)
def _scatter_add(tgt, idx, src, axis=0):
    return tgt.at[idx].add(src)
def _segment_sum(src, seg, n):
    return jax.ops.segment_sum(src, seg, n)
class _Rng:
    def __init__(self, key):
        self._k = key
    def _next(self):
        self._k, sub = jax.random.split(self._k)
        return sub
    def normal(self, shape):
        return jax.random.normal(self._next(), shape, dtype=jnp.bfloat16)
    def randint(self, lo, hi, shape):
        return jax.random.randint(self._next(), shape, lo, hi, dtype=jnp.int32)
    def uniform(self, shape, lo=0.0, hi=1.0):
        return jax.random.uniform(self._next(), shape, jnp.bfloat16, lo, hi)
    def permutation(self, n):
        return jax.random.permutation(self._next(), n)


kernel_name = 'sequential_preLN__sliding_local_dilated__dense_activation_mish__prompt'

def setup_inputs():
    _rng = _Rng(jax.random.key(int.from_bytes(__import__("os").urandom(4), "little")))
    _w = (lambda a: (lambda t: t.astype(jnp.bfloat16) if jnp.issubdtype(t.dtype, jnp.floating) else t)(jnp.asarray(a)))
    def _A_setup():
        B, S, D = 1, 2048, 512
        return {
            "x": _w((lambda *s: _rng.normal(s) * 0.05)(B, S, D)),
            "wqkv": _w((lambda *s: _rng.normal(s) * 0.05)(D, 3 * D)),
            "wo": _w((lambda *s: _rng.normal(s) * 0.05)(D, D)),
        }
    _A_in = _A_setup()

    def _B_setup():
        B, S, D, F = 1, 2048, 512, 1376
        return {
            "x": _w((lambda *s: _rng.normal(s) * 0.05)(B, S, D)),
            "w1": _w((lambda *s: _rng.normal(s) * 1.6)(D, F) * (D ** -0.5)),
            "b1": _w((lambda *s: _rng.normal(s) * 0.1)(F)),
            "w2": _w((lambda *s: _rng.normal(s) * 0.1)(F, D) * (F ** -0.5)),
        }
    _B_in = _B_setup()

    return {
        "A_x": _A_in["x"],
        "A_wqkv": _A_in["wqkv"],
        "A_wo": _A_in["wo"],
        "B_x": _B_in["x"],
        "B_w1": _B_in["w1"],
        "B_b1": _B_in["b1"],
        "B_w2": _B_in["w2"],
    }

def reference(A_x, A_wqkv, A_wo, B_x, B_w1, B_b1, B_w2):
    def _A_ref(x, wqkv, wo):
        B, S, D = x.shape
        H = 32; Dh = D // H
        W, dil = 8, 2
        qkv = (lambda x, *d: x.transpose(*d))((x @ wqkv).reshape(B, S, 3, H, Dh), 2, 0, 3, 1, 4)
        q, k, v = qkv[0], qkv[1], qkv[2]
        scale = Dh ** -0.5
        pos = jnp.arange(S)
        off = jnp.arange(W) * dil
        idx = pos[:, None] - off[None, :]
        mask = idx >= 0
        idx_c = jnp.where(mask, idx, 0).reshape(-1)
        kg = k[:, :, idx_c, :].reshape(B, H, S, W, Dh)
        vg = v[:, :, idx_c, :].reshape(B, H, S, W, Dh)
        logits = jnp.einsum("bhsd,bhswd->bhsw", q, kg) * scale
        logits = jnp.where(mask[None, None, :, :], logits, -1e9)
        attn = _softmax(logits, axis=-1)
        o = jnp.einsum("bhsw,bhswd->bhsd", attn, vg)
        return (lambda x, *d: x.transpose(*d))(o, 0, 2, 1, 3).reshape(B, S, D) @ wo

    def _B_ref(x, w1, b1, w2):
        h = jnp.einsum("bsd,df->bsf", x, w1) + b1
        sp = jnp.log1p(jnp.exp(-jnp.abs(h))) + jnp.where(h > 0, h, jnp.zeros_like(h))
        act = h * jnp.tanh(sp)
        return jnp.einsum("bsf,fd->bsd", act, w2)

    x = A_x
    h = x + _A_ref(_layernorm(x, axis=-1), A_wqkv, A_wo)
    h2 = h + _B_ref(_layernorm(h, axis=-1), B_w1, B_b1, B_w2)
    return h2
```

```python
import jax
import jax.numpy as jnp
import jax.experimental.pallas as pl
import jax.experimental.pallas.tpu as pltpu

S, D, H, DH, F = 2048, 512, 32, 16, 1376
W, DIL = 8, 2
HALO = 16
T = 256
VMEM_MB = 64


def _ln(x):
    m = jnp.mean(x, axis=-1, keepdims=True)
    xc = x - m
    v = jnp.mean(xc * xc, axis=-1, keepdims=True)
    return xc * jax.lax.rsqrt(v + 1e-5)


def _kernel(x_ref, wqkv_hbm, wo_hbm, w1t_hbm, b1_ref, w2_hbm, o_ref,
            wqkv_ref, wo_ref, w1t_ref, w2_ref, sems, wqkv_p, wo_p, kbuf, vbuf):
    i = pl.program_id(0)
    f32 = jnp.float32
    bf16 = jnp.bfloat16

    @pl.when(i == 0)
    def _():
        cps = [pltpu.make_async_copy(src, dst, sems.at[n]) for n, (src, dst) in enumerate(
            [(wqkv_hbm, wqkv_ref), (wo_hbm, wo_ref), (w1t_hbm, w1t_ref), (w2_hbm, w2_ref)])]
        for cp in cps:
            cp.start()
        cps[0].wait()
        r = jax.lax.broadcasted_iota(jnp.int32, (D, D), 0)
        c = jax.lax.broadcasted_iota(jnp.int32, (D, D), 1)
        pm = jnp.where(c == (r % DH) * H + r // DH, 1.0, 0.0).astype(bf16)
        for j in range(3):
            wqkv_p[:, j * D:(j + 1) * D] = jnp.dot(
                wqkv_ref[:, j * D:(j + 1) * D], pm, preferred_element_type=f32).astype(bf16)
        cps[1].wait()
        pmt = jnp.where(r == (c % DH) * H + c // DH, 1.0, 0.0).astype(bf16)
        wo_p[...] = jnp.dot(pmt, wo_ref[...], preferred_element_type=f32).astype(bf16)
        kbuf[0:HALO, :] = jnp.zeros((HALO, D), f32)
        vbuf[0:HALO, :] = jnp.zeros((HALO, D), f32)
        cps[2].wait()
        cps[3].wait()

    @pl.when(i > 0)
    def _():
        kbuf[0:HALO, :] = kbuf[T:T + HALO, :]
        vbuf[0:HALO, :] = vbuf[T:T + HALO, :]

    x = x_ref[...].astype(f32)
    xn = _ln(x).astype(bf16)
    qkv = jnp.dot(xn, wqkv_p[...], preferred_element_type=f32)
    q = qkv[:, :D] * (DH ** -0.5)
    kbuf[HALO:HALO + T, :] = qkv[:, D:2 * D]
    vbuf[HALO:HALO + T, :] = qkv[:, 2 * D:]

    row = i * T + jax.lax.broadcasted_iota(jnp.int32, (T, 128), 0)
    logits = []
    for w in range(W):
        ks = kbuf[HALO - DIL * w:HALO - DIL * w + T, :]
        p = q * ks
        r = p[:, 0:128] + p[:, 128:256] + p[:, 256:384] + p[:, 384:512]
        r = r + pltpu.roll(r, 64, 1)
        r = r + pltpu.roll(r, 32, 1)
        if w > 0:
            r = jnp.where(row >= DIL * w, r, -1e9)
        logits.append(r)
    m = logits[0]
    for w in range(1, W):
        m = jnp.maximum(m, logits[w])
    es = [jnp.exp(l - m) for l in logits]
    ssum = es[0]
    for w in range(1, W):
        ssum = ssum + es[w]
    inv = 1.0 / ssum
    cols = []
    for c in range(4):
        acc = None
        for w in range(W):
            vs = vbuf[HALO - DIL * w:HALO - DIL * w + T, c * 128:(c + 1) * 128]
            t = es[w] * vs
            acc = t if acc is None else acc + t
        cols.append(acc * inv)
    o = jnp.concatenate(cols, axis=1).astype(bf16)
    h = x + jnp.dot(o, wo_p[...], preferred_element_type=f32)
    hn = _ln(h).astype(bf16)
    z = jax.lax.dot_general(hn, w1t_ref[...], (((1,), (1,)), ((), ())),
                            preferred_element_type=f32) + b1_ref[...].astype(f32)
    u = jnp.exp(-jnp.abs(z))
    pos = z > 0
    n = jnp.where(pos, 1.0 + 2.0 * u, u * (u + 2.0))
    d = n + jnp.where(pos, 2.0 * u * u, 2.0)
    act = (z * n / d).astype(bf16)
    y = h + jnp.dot(act, w2_ref[...], preferred_element_type=f32)
    o_ref[...] = y.astype(o_ref.dtype)


@jax.jit
def pallas_sequential_preLN__sliding_local_dilated__dense_activation_mish__prompt_kernel(
    A_x: jax.Array,
    A_wqkv: jax.Array,
    A_wo: jax.Array,
    B_x: jax.Array,
    B_w1: jax.Array,
    B_b1: jax.Array,
    B_w2: jax.Array,
):
    x = A_x.reshape(S, D)
    b1 = B_b1.reshape(1, F)
    const = lambda i: (0, 0)
    out = pl.pallas_call(
        _kernel,
        grid=(S // T,),
        in_specs=[
            pl.BlockSpec((T, D), lambda i: (i, 0)),
            pl.BlockSpec(memory_space=pl.ANY),
            pl.BlockSpec(memory_space=pl.ANY),
            pl.BlockSpec(memory_space=pl.ANY),
            pl.BlockSpec((1, F), const),
            pl.BlockSpec(memory_space=pl.ANY),
        ],
        out_specs=pl.BlockSpec((T, D), lambda i: (i, 0)),
        out_shape=jax.ShapeDtypeStruct((S, D), jnp.bfloat16),
        scratch_shapes=[
            pltpu.VMEM((D, 3 * D), jnp.bfloat16),
            pltpu.VMEM((D, D), jnp.bfloat16),
            pltpu.VMEM((F, D), jnp.bfloat16),
            pltpu.VMEM((F, D), jnp.bfloat16),
            pltpu.SemaphoreType.DMA((4,)),
            pltpu.VMEM((D, 3 * D), jnp.bfloat16),
            pltpu.VMEM((D, D), jnp.bfloat16),
            pltpu.VMEM((T + HALO, D), jnp.float32),
            pltpu.VMEM((T + HALO, D), jnp.float32),
        ],
        compiler_params=pltpu.CompilerParams(
            dimension_semantics=("arbitrary",),
            vmem_limit_bytes=VMEM_MB * 1024 * 1024,
        ),
    )(x, A_wqkv, A_wo, B_w1.T, b1, B_w2)
    return out.reshape(1, S, D)
```

```python
import jax
import jax.numpy as jnp
import jax.experimental.pallas as pl
import jax.experimental.pallas.tpu as pltpu

S, D, H, DH, F = 2048, 512, 32, 16, 1376
W, DIL = 8, 2
HALO = 16
T = 512
VMEM_MB = 64


def _ln(x):
    m = jnp.mean(x, axis=-1, keepdims=True)
    xc = x - m
    v = jnp.mean(xc * xc, axis=-1, keepdims=True)
    return xc * jax.lax.rsqrt(v + 1e-5)


def _kernel(x_ref, wqkv_hbm, wo_hbm, w1t_hbm, b1_ref, w2_hbm, o_ref,
            wqkv_ref, wo_ref, w1t_ref, w2_ref, sems, wqkv_p, wo_p, kbuf, vbuf):
    i = pl.program_id(0)
    f32 = jnp.float32
    bf16 = jnp.bfloat16

    @pl.when(i == 0)
    def _():
        cps = [pltpu.make_async_copy(src, dst, sems.at[n]) for n, (src, dst) in enumerate(
            [(wqkv_hbm, wqkv_ref), (wo_hbm, wo_ref), (w1t_hbm, w1t_ref), (w2_hbm, w2_ref)])]
        for cp in cps:
            cp.start()
        cps[0].wait()
        r = jax.lax.broadcasted_iota(jnp.int32, (D, D), 0)
        c = jax.lax.broadcasted_iota(jnp.int32, (D, D), 1)
        hit = c == (r % DH) * H + r // DH
        pm = jnp.where(hit, 1.0, 0.0).astype(bf16)
        pmq = jnp.where(hit, DH ** -0.5, 0.0).astype(bf16)
        for j in range(3):
            wqkv_p[:, j * D:(j + 1) * D] = jnp.dot(
                wqkv_ref[:, j * D:(j + 1) * D], pmq if j == 0 else pm,
                preferred_element_type=f32).astype(bf16)
        cps[1].wait()
        pmt = jnp.where(r == (c % DH) * H + c // DH, 1.0, 0.0).astype(bf16)
        wo_p[...] = jnp.dot(pmt, wo_ref[...], preferred_element_type=f32).astype(bf16)
        kbuf[0:HALO, :] = jnp.zeros((HALO, D), f32)
        vbuf[0:HALO, :] = jnp.zeros((HALO, D), f32)
        cps[2].wait()
        cps[3].wait()

    @pl.when(i > 0)
    def _():
        kbuf[0:HALO, :] = kbuf[T:T + HALO, :]
        vbuf[0:HALO, :] = vbuf[T:T + HALO, :]

    x = x_ref[...].astype(f32)
    xn = _ln(x).astype(bf16)
    qkv = jnp.dot(xn, wqkv_p[...], preferred_element_type=f32)
    q = qkv[:, :D]
    kbuf[HALO:HALO + T, :] = qkv[:, D:2 * D]
    vbuf[HALO:HALO + T, :] = qkv[:, 2 * D:]

    row = i * T + jax.lax.broadcasted_iota(jnp.int32, (T, 128), 0)
    kwin = [kbuf[HALO - 8 - DIL * a:HALO - DIL * a + T, :] for a in range(4)]
    vwin = [vbuf[HALO - 8 - DIL * a:HALO - DIL * a + T, :] for a in range(4)]
    kshift = lambda w: kwin[w % 4][8:8 + T] if w < 4 else kwin[w % 4][0:T]
    vshift = lambda w: vwin[w % 4][8:8 + T] if w < 4 else vwin[w % 4][0:T]
    logits = []
    for w in range(W):
        ks = kshift(w)
        p = q * ks
        r = p[:, 0:128] + p[:, 128:256] + p[:, 256:384] + p[:, 384:512]
        r = r + pltpu.roll(r, 64, 1)
        r = r + pltpu.roll(r, 32, 1)
        if w > 0:
            r = jnp.where(row >= DIL * w, r, -1e9)
        logits.append(r)
    m = logits[0]
    for w in range(1, W):
        m = jnp.maximum(m, logits[w])
    es = [jnp.exp(l - m) for l in logits]
    ssum = es[0]
    for w in range(1, W):
        ssum = ssum + es[w]
    inv = 1.0 / ssum
    cols = []
    for c in range(4):
        acc = None
        for w in range(W):
            vs = vshift(w)[:, c * 128:(c + 1) * 128]
            t = es[w] * vs
            acc = t if acc is None else acc + t
        cols.append(acc * inv)
    o = jnp.concatenate(cols, axis=1).astype(bf16)
    h = x + jnp.dot(o, wo_p[...], preferred_element_type=f32)
    hn = _ln(h).astype(bf16)
    z = jax.lax.dot_general(hn, w1t_ref[...], (((1,), (1,)), ((), ())),
                            preferred_element_type=f32) + b1_ref[...].astype(f32)
    u = jnp.exp(-jnp.abs(z))
    pos = z > 0
    n = jnp.where(pos, 1.0 + 2.0 * u, u * (u + 2.0))
    d = n + jnp.where(pos, 2.0 * u * u, 2.0)
    act = (z * n / d).astype(bf16)
    y = h + jnp.dot(act, w2_ref[...], preferred_element_type=f32)
    o_ref[...] = y.astype(o_ref.dtype)


@jax.jit
def pallas_sequential_preLN__sliding_local_dilated__dense_activation_mish__prompt_kernel(
    A_x: jax.Array,
    A_wqkv: jax.Array,
    A_wo: jax.Array,
    B_x: jax.Array,
    B_w1: jax.Array,
    B_b1: jax.Array,
    B_w2: jax.Array,
):
    x = A_x.reshape(S, D)
    b1 = B_b1.reshape(1, F)
    const = lambda i: (0, 0)
    out = pl.pallas_call(
        _kernel,
        grid=(S // T,),
        in_specs=[
            pl.BlockSpec((T, D), lambda i: (i, 0)),
            pl.BlockSpec(memory_space=pl.ANY),
            pl.BlockSpec(memory_space=pl.ANY),
            pl.BlockSpec(memory_space=pl.ANY),
            pl.BlockSpec((1, F), const),
            pl.BlockSpec(memory_space=pl.ANY),
        ],
        out_specs=pl.BlockSpec((T, D), lambda i: (i, 0)),
        out_shape=jax.ShapeDtypeStruct((S, D), jnp.bfloat16),
        scratch_shapes=[
            pltpu.VMEM((D, 3 * D), jnp.bfloat16),
            pltpu.VMEM((D, D), jnp.bfloat16),
            pltpu.VMEM((F, D), jnp.bfloat16),
            pltpu.VMEM((F, D), jnp.bfloat16),
            pltpu.SemaphoreType.DMA((4,)),
            pltpu.VMEM((D, 3 * D), jnp.bfloat16),
            pltpu.VMEM((D, D), jnp.bfloat16),
            pltpu.VMEM((T + HALO, D), jnp.float32),
            pltpu.VMEM((T + HALO, D), jnp.float32),
        ],
        compiler_params=pltpu.CompilerParams(
            dimension_semantics=("arbitrary",),
            vmem_limit_bytes=VMEM_MB * 1024 * 1024,
        ),
    )(x, A_wqkv, A_wo, B_w1.T, b1, B_w2)
    return out.reshape(1, S, D)
```
